```python
import os as _os
_os.environ.setdefault('JAX_PLATFORMS', 'cpu')
import jax
import jax.numpy as jnp

def _softmax(x, axis=-1):
    return jax.nn.softmax(x, axis=axis)

def _gelu(x):
    return jax.nn.gelu(x, approximate=True)

def _silu(x):
    return jax.nn.silu(x)

def _sigmoid(x):
    return jax.nn.sigmoid(x)

def _layernorm(x, axis=-1, eps=1e-05):
    m = jnp.mean(x, axis=axis, keepdims=True)
    v = jnp.var(x, axis=axis, keepdims=True)
    return (x - m) / jnp.sqrt(v + eps)

def _scatter_add(tgt, idx, src, axis=0):
    return tgt.at[idx].add(src)

def _segment_sum(src, seg, n):
    return jax.ops.segment_sum(src, seg, n)

class _Rng:

    def __init__(self, key):
        self._k = key

    def _next(self):
        self._k, sub = jax.random.split(self._k)
        return sub

    def normal(self, shape):
        return jax.random.normal(self._next(), shape, dtype=jnp.bfloat16)

    def randint(self, lo, hi, shape):
        return jax.random.randint(self._next(), shape, lo, hi, dtype=jnp.int32)

    def uniform(self, shape, lo=0.0, hi=1.0):
        return jax.random.uniform(self._next(), shape, jnp.bfloat16, lo, hi)

    def permutation(self, n):
        return jax.random.permutation(self._next(), n)
kernel_name = 'sequential_preLN__memory_aug_recurrent_mem_tr__mixer_token_mlp__prompt'

def setup_inputs():
    _rng = _Rng(jax.random.key(int.from_bytes(__import__("os").urandom(4), "little")))
    _w = lambda a: (lambda t: t.astype(jnp.bfloat16) if jnp.issubdtype(t.dtype, jnp.floating) else t)(jnp.asarray(a))

    def _A_setup():
        B, S, Dm = (1, 2048, 448)
        H, Dh = (16, 256)
        M, seg = (8, 32)
        seg = min(seg, S)
        S = S // seg * seg
        return {'x': _w((lambda *s: _rng.normal(s) * 0.05)(B, S, Dm)), 'mem0': _w((lambda *s: _rng.normal(s) * 0.2)(B, M, Dm)), 'Wq': _w((lambda *s: _rng.normal(s) * 1.6)(Dm, H, Dh) * Dm ** (-0.5)), 'Wk': _w((lambda *s: _rng.normal(s) * 1.6)(Dm, H, Dh) * Dm ** (-0.5)), 'Wv': _w((lambda *s: _rng.normal(s) * 0.2)(Dm, H, Dh) * Dm ** (-0.5)), 'Wo': _w((lambda *s: _rng.normal(s) * 0.2)(H, Dh, Dm) * (H * Dh) ** (-0.5)), 'seg_len': seg}
    _A_in = _A_setup()

    def _B_setup():
        B, S, D, F = (1, 2048, 448, 1792)
        return {'x': _w((lambda *s: _rng.normal(s) * 0.05)(B, S, D)), 'w1': _w((lambda *s: _rng.normal(s) * 0.2)(S, F) * S ** (-0.5)), 'b1': _w((lambda *s: _rng.normal(s) * 0.2)(F) * 0.02), 'w2': _w((lambda *s: _rng.normal(s) * 0.2)(F, S) * F ** (-0.5)), 'b2': _w((lambda *s: _rng.normal(s) * 0.05)(S) * 0.02)}
    _B_in = _B_setup()
    return {'A_x': _A_in['x'], 'A_mem0': _A_in['mem0'], 'A_Wq': _A_in['Wq'], 'A_Wk': _A_in['Wk'], 'A_Wv': _A_in['Wv'], 'A_Wo': _A_in['Wo'], 'A_seg_len': _A_in['seg_len'], 'B_x': _B_in['x'], 'B_w1': _B_in['w1'], 'B_b1': _B_in['b1'], 'B_w2': _B_in['w2'], 'B_b2': _B_in['b2']}

def reference(A_x, A_mem0, A_Wq, A_Wk, A_Wv, A_Wo, A_seg_len, B_x, B_w1, B_b1, B_w2, B_b2):

    def _A_ref(x, mem0, Wq, Wk, Wv, Wo, seg_len):
        B, S, Dm = x.shape
        H, Dh = (Wq.shape[1], Wq.shape[2])
        M = mem0.shape[1]
        scale = Dh ** (-0.5)
        n_seg = S // seg_len
        L = M + seg_len
        idx = jnp.arange(L)
        mask = (idx[:, None] < M) | (idx[:, None] >= idx[None, :])
        mem = mem0
        outs = []
        for s in range(n_seg):
            xs = x[:, s * seg_len:(s + 1) * seg_len, :].copy()
            h = jnp.concatenate([mem, xs], axis=1)
            q = jnp.einsum('btd,dhe->bhte', h, Wq)
            k = jnp.einsum('btd,dhe->bhte', h, Wk)
            v = jnp.einsum('btd,dhe->bhte', h, Wv)
            scores = jnp.einsum('bhqe,bhke->bhqk', q, k) * scale
            scores = jnp.where(mask[None, None], scores, -1000000000.0)
            p = _softmax(scores, axis=-1)
            o = jnp.einsum('bhqk,bhke->bhqe', p, v)
            o = jnp.einsum('bhte,hed->btd', o, Wo)
            mem = o[:, :M, :].copy()
            outs.append(o[:, M:, :])
        return jnp.concatenate(outs, axis=1)

    def _B_ref(x, w1, b1, w2, b2):
        B, S, D = x.shape
        h = _layernorm(x, axis=-1)
        u = jnp.einsum('bsd,sf->bdf', h, w1) + b1
        u = _gelu(u)
        y = jnp.einsum('bdf,fs->bds', u, w2) + b2
        return (lambda x, *d: x.transpose(*d))(y, 0, 2, 1)
    x = A_x
    h = x + _A_ref(_layernorm(x, axis=-1), A_mem0, A_Wq, A_Wk, A_Wv, A_Wo, A_seg_len)
    h2 = h + _B_ref(_layernorm(h, axis=-1), B_w1, B_b1, B_w2, B_b2)
    return h2
```

```python
import functools

import jax
import jax.experimental.pallas as pl
import jax.experimental.pallas.tpu as pltpu
import jax.numpy as jnp
from jax import lax

F32, BF16, U32 = jnp.float32, jnp.bfloat16, jnp.uint32

D = 448
S = 2048
H = 16
E = 256
M = 8
SEG = 32
L = M + SEG
F = 1792
BLK = 128
NSEG = BLK // SEG
NBLK = S // BLK
JB = L // 8
DT = 3
D1 = 128 * DT
D2 = D - D1
HP = H // 2
NP = 15
OUT_COLS = 256
EPS = 1e-5
NEG = -1000000000.0

NT = (((1,), (1,)), ((), ()))
NN = (((1,), (0,)), ((), ()))


def _dot(a, b, dims=NN):
    return lax.dot_general(a, b, dims, preferred_element_type=F32)


def _words(x):
    return pltpu.bitcast(x, U32)


def _bf16(x):
    return pltpu.bitcast(x, BF16)


def _cat(xs, axis):
    return xs[0] if len(xs) == 1 else jnp.concatenate(xs, axis=axis)


def _tile(x, t):
    return x[:, 128 * t:128 * t + 128]


def _tiles(x):
    return [_tile(x, t) for t in range(DT)]


def _layernorm_columns(x):
    m = jnp.sum(x, axis=0, keepdims=True) * (1.0 / D)
    c = x - m
    v = jnp.sum(c * c, axis=0, keepdims=True) * (1.0 / D)
    return c * lax.rsqrt(v + EPS)


def _reduce_groups(x, op, lane):
    terms = [x] + [jnp.where(lane % 8 + k < 8, pltpu.roll(x, 128 - k, 1), pltpu.roll(x, 8 - k, 1))
                   for k in range(1, 8)]
    while len(terms) > 1:
        terms = [op(a, b) for a, b in zip(terms[::2], terms[1::2])]
    return terms[0]


def _weight_forms(w):
    (w11, w12, w13), (w21, w22, w23), (w31, w32, w33) = w
    return {1: w11 - w31 - w12, 2: w11 - w21 - w13, 3: w22 - w21 - w32, 4: w22 - w12 - w23, 5: w33 - w31 - w23,
            6: w33 - w32 - w13, 7: w21, 8: w12 - w21, 9: w12, 10: w23, 11: w32 - w23, 12: w32, 13: w13 - w31,
            14: w13, 15: w31}


def _token_forms(a, b):
    (a1, a2, a3), (b1, b2, b3) = a, b
    b12, a23 = b1 + b2, a2 + a3
    return {1: a1, 2: a1 + b1, 3: a2, 4: b2, 5: a3 + b3, 6: b3, 7: a1 + a2 + b12, 8: a1 + b12, 9: b12,
            10: a23 + b2 + b3, 11: a23 + b3, 12: a23, 13: a1 - b3, 14: b1 + b3, 15: a1 + a3}


TOKEN_PRODUCTS = ((1, 3, 5, 7, 9, 10, 12, 15), (2, 4, 6, 8, 11, 13, 14))


def _first_half(p):
    z23 = p[10] - p[12]
    z21 = p[1] - p[9]
    z = [z21 + p[15], p[3] - p[9] + p[12], p[5] + p[12] + p[15], z21, z23 + p[9], z23]
    return [z[0] + p[7], z[1] + p[7]] + z[2:]


def _second_half(p, z):
    t = p[6] + p[11]
    return ([z[0] + p[8], z[1] + p[8], z[2] - t + p[13]],
            [p[2] - p[8] - z[3] + p[13] + p[14], z[4] + p[4] + p[11], z[5] + t + p[14]])


STEP_PRODUCTS = ((1, 3, 5, 10, 12, 13, 9, 7, 15), (2, 7, 4, 6, 8, 11, 13, 10, 14))


def _memory_forms(m, odd):
    m1, m2, m3 = m
    m12, m13, m23 = m1 + m2, m1 + m3, m2 + m3
    if odd:
        return {2: m1, 4: m2, 6: m3, 7: m12, 8: m12, 10: m23, 11: m3, 13: m3, 14: m13}
    return {1: m1, 3: m2, 5: m3, 7: m2, 9: m1, 10: m23, 12: m23, 13: m1, 15: m13}


def _memory_out(p, odd):
    if odd:
        t = p[10] + p[11]
        return [p[2] + p[7] + p[14] - p[13], p[4] + p[7] + p[8] + t, p[6] + p[14] + t]
    t = p[7] + p[9]
    return [p[1] + t + p[15], p[3] + t + p[12], p[5] + p[10] + p[13] + p[15]]


EXTRA_GROUPS = ((("k", 0), ("q", 0), ("k", 1)), (("q", 1), ("k", 2), ("q", 2)), (("v", 0), ("v", 1), ("v", 2)))
EXTRA_SINGLES = (("k", 3), ("q", 3), ("v", 3))

SCHEDULE = (
    "q S4 K01 X0 K12 S31 X1 K23 t08 K34 S2 K451 S11 K562 K67 K78 V013 V12 S0 V24 M0 V45 V58 x M1 z08 P15 b08 P01 M2 M3",
    "K01 X0 K12 K23 S3 S4 q K34 X1 K450 S1 t08 K56 S21 K671 K782 T0 T1 V013 V12 S0 M0 V23 V346 V454 V56 V675 V78 x "
    "M16 M34 z08 P15 b08 P01 M2",
)


def _kernel(xt_hbm, mem0_ref, wq_hbm, wk_hbm, wv_hbm, wot_hbm, w1_hbm, b1_ref, w2_hbm, b2_ref,
            out_hbm,
            xt_v, wq_v, wk_v, wv_v, wot_v, w1_v, w2_v,
            kform, vform, xform, xplain, wq2, wv2, x_cur, x_next, o_s, ht_s, g_s, u_s,
            k_mem, v_mem, k_tok, v_tok, q_tok, k_half, v_half, x_half, kt_mem, kt_tok, a_s, b2_s, out_v,
            wsems, lsems, ysems):
    def heads(hf):
        return pl.ds(pl.multiple_of(8 * hf, 8), 8)

    def value_copies(hf):
        return [pltpu.make_async_copy(wv_hbm.at[:, heads(hf), :], wv_v.at[hf], wsems.at[5 * hf])] + [
            pltpu.make_async_copy(wot_hbm.at[pl.ds(8 * hf + 4 * c, 4)], wot_v.at[hf, pl.ds(4 * c, 4)],
                                  wsems.at[5 * hf + 1 + c]) for c in range(2)]

    def key_copies(hf):
        return [pltpu.make_async_copy(wq_hbm.at[:, heads(hf), :], wq_v.at[hf], wsems.at[5 * hf + 3]),
                pltpu.make_async_copy(wk_hbm.at[:, heads(hf), :], wk_v.at[hf], wsems.at[5 * hf + 4])]

    x_head = pltpu.make_async_copy(xt_hbm.at[:, pl.ds(0, BLK)], xt_v.at[:, pl.ds(0, BLK)], lsems.at[0])
    x_rest = pltpu.make_async_copy(xt_hbm.at[:, pl.ds(BLK, S - BLK)], xt_v.at[:, pl.ds(BLK, S - BLK)], lsems.at[1])
    w1_head = pltpu.make_async_copy(w1_hbm.at[pl.ds(0, BLK)], w1_v.at[pl.ds(0, BLK)], lsems.at[2])
    w1_rest = pltpu.make_async_copy(w1_hbm.at[pl.ds(BLK, S - BLK)], w1_v.at[pl.ds(BLK, S - BLK)], lsems.at[3])
    w2_all = pltpu.make_async_copy(w2_hbm, w2_v, lsems.at[4])
    queue = [x_head] + value_copies(0) + value_copies(1) + key_copies(0) + key_copies(1) + [x_rest, w1_head]

    def request(i, carry):
        for k, copy in enumerate(queue):
            pl.when(i == k)(copy.start)
        return carry

    lax.fori_loop(0, len(queue), request, 0)

    def clear(i, carry):
        u_s[pl.ds(pl.multiple_of(i * 32, 32), 32), :] = jnp.zeros((32, F), F32)
        return carry

    lax.fori_loop(0, D // 32, clear, 0)
    o_s[...] = jnp.zeros(o_s.shape, F32)
    b2_s[...] = jnp.broadcast_to(b2_ref[...].astype(F32).reshape(1, S), b2_s.shape)

    def by_head(w):
        w = jnp.swapaxes(w, 0, 1)
        return [w[hd] for hd in range(8)]

    def put_forms(form, i, columns):
        blocks = [[c[128 * k:128 * k + 128] for c in columns] for k in range(DT)]
        for p, t in _weight_forms(blocks).items():
            form[i, p - 1] = _words(t.astype(BF16))

    def put_extras(hf, columns):
        for g, group in enumerate(EXTRA_GROUPS):
            if group[0] in columns:
                put_forms(xform, len(EXTRA_GROUPS) * hf + g, [columns[c] for c in group])
        for g, c in enumerate(EXTRA_SINGLES):
            if c in columns:
                xplain[len(EXTRA_SINGLES) * hf + g] = _words(columns[c].astype(BF16))

    def fold_pair(ls, rs, a, form):
        full = [_dot(l, r[:D1], NT) for l, r in zip(ls, rs)]
        rp = jnp.concatenate([r[D1:] for r in rs], axis=0)
        lane = lax.broadcasted_iota(jnp.int32, (D, 128), 1)
        shared = jnp.where(lane < D2, *[_dot(l, rp, NT) for l in ls])
        for b, y in enumerate(full):
            put_forms(form, 2 * a + b, _tiles(y))
        tails = [jnp.concatenate([_tile(y[D1:], dt) for y in full], axis=0) for dt in range(DT)]
        tails.append(jnp.concatenate([shared[D1:], pltpu.roll(shared[D1:], D2, 1)], axis=0))
        return shared[:D1], [t.astype(BF16) for t in tails]

    def fold_values(hf, carry):
        arrivals = value_copies(hf)
        arrivals[0].wait()
        wv = by_head(wv_v[hf])
        extras = {}
        for k in range(HP // 2):
            a = 4 * hf + k
            if k % 2 == 0:
                arrivals[1 + k // 2].wait()
            extras["v", k], tails = fold_pair(wv[2 * k:2 * k + 2], [wot_v[hf, 2 * k + b] for b in range(2)], a, vform)
            for dt, t in enumerate(tails):
                wv2[dt, a] = _words(t)
        put_extras(hf, extras)
        return carry

    def fold_keys(hf, carry):
        for copy in key_copies(hf):
            copy.wait()
        wq, wk = by_head(wq_v[hf]), by_head(wk_v[hf])
        extras = {}
        for k in range(HP // 2):
            a = 4 * hf + k
            extras["k", k], tails = fold_pair(wk[2 * k:2 * k + 2], wq[2 * k:2 * k + 2], a, kform)
            extras["q", k] = jnp.concatenate([t.T.astype(F32) for t in tails[:DT]], axis=0)
            wq2[a] = _words(tails[DT].T[:D2])
        put_extras(hf, extras)
        first_tokens("K", hf)
        first_tokens("X", hf)
        return carry

    def normalized_tokens(blk):
        c0 = pl.multiple_of(blk * BLK, BLK)
        return _layernorm_columns(xt_v[:, pl.ds(c0, BLK)].astype(F32)).T

    def mixer_input(blk):
        c0 = pl.multiple_of(blk * BLK, BLK)
        h = xt_v[:, pl.ds(c0, BLK)].astype(F32) + o_s[...].T
        ht_s[:, pl.ds(c0, BLK)] = h
        return _layernorm_columns(_layernorm_columns(h)).astype(BF16)

    def put_rows(dst, a, y0, y1):
        for j in range(y0.shape[0] // 8):
            t = jnp.concatenate([y0[8 * j:8 * j + 8], y1[8 * j:8 * j + 8]], axis=0).astype(BF16)
            dst(j)[pl.ds(pl.multiple_of(16 * a, 16), 16), :] = t

    def put_extra(slot, hf, column, y):
        kind, a = column[0], 4 * hf + column[1]
        if kind == "q":
            q_tok[slot, a] = y
        else:
            dst = k_tok if kind == "k" else v_tok
            put_rows(lambda j: dst.at[slot, DT, j], a, y, pltpu.roll(y, D2, 1))

    def turn_keys(slot):
        ts = [_words(_cat([k_tok[slot, dt, j].T for dt in range(DT + 1)], 0)[:D]) for j in range(JB - 1)]
        for j, t in enumerate(ts):
            kt_tok[slot, j] = t
        return ts

    sides = {"K": (kform, k_mem, k_tok, k_half), "V": (vform, v_mem, v_tok, v_half)}

    def first_tokens(side, hf):
        tok = _token_forms(_tiles(x_cur[:SEG]), _tiles(x_cur[SEG:2 * SEG]))

        def project(form, i):
            p = {q: _dot(tok[q], _bf16(form[i, q - 1])) for q in tok}
            return _second_half(p, _first_half(p))

        if side == "X":
            for g, group in enumerate(EXTRA_GROUPS):
                for slot, ys in enumerate(project(xform, len(EXTRA_GROUPS) * hf + g)):
                    for column, y in zip(group, ys):
                        put_extra(slot, hf, column, y)
            for g, column in enumerate(EXTRA_SINGLES):
                y = _dot(x_cur[:2 * SEG, :D1], _bf16(xplain[len(EXTRA_SINGLES) * hf + g]))
                for slot in range(2):
                    put_extra(slot, hf, column, y[SEG * slot:SEG * slot + SEG])
            return
        form, _, dst, _ = sides[side]
        for k in range(HP // 2):
            a = 4 * hf + k
            ys = [project(form, 2 * a + b) for b in range(2)]
            for slot in range(2):
                for dt in range(DT):
                    put_rows(lambda j: dst.at[slot, dt, j], a, ys[0][slot][dt], ys[1][slot][dt])

    x_head.wait()
    x_cur[...] = normalized_tokens(0)
    lax.fori_loop(0, 2, fold_values, 0)
    lax.fori_loop(0, 2, fold_keys, 0)
    for hf in range(2):
        first_tokens("V", hf)
    for slot in range(2):
        turn_keys(slot)
    x_rest.wait()
    w1_head.wait()
    w1_rest.start()

    lane = lax.broadcasted_iota(jnp.int32, (L, 128), 1)
    row = lax.broadcasted_iota(jnp.int32, (L, 128), 0)
    pair_of_lane = lane >> 4

    def step(i, h, ahead, mix, always):
        odd = i % 2
        slots = [(i - odd + 2) % NSEG, (i - odd + 3) % NSEG]
        tok = _token_forms(_tiles(ahead[:SEG]), _tiles(ahead[SEG:]))
        mem = _memory_forms(_tiles(h[:M]), odd)
        lhs = {p: jnp.concatenate([mem[p], tok[p]], axis=0) if p in TOKEN_PRODUCTS[odd] else mem[p] for p in mem}
        x2 = jnp.concatenate([h[:, D1:], jnp.zeros((L, 128 - D2), F32)], axis=1)
        x2r = pltpu.roll(x2, D2, 1)
        x2g = [jnp.concatenate([x2[8 * j:8 * j + 8], x2r[8 * j:8 * j + 8]], axis=0).astype(BF16)
               for j in range(JB)] + [jnp.zeros((16, 128), BF16)] * (HP - JB)
        env = {"marks": []}

        def after(x, dep):
            n = -(-x.shape[1] // 128)
            head = jnp.where(always[:, :x.shape[1]], x[:8], _cat([dep[:8]] * n, 1)[:, :x.shape[1]])
            return jnp.concatenate([head, x[8:]], axis=0) if x.shape[0] > 8 else head

        def live(x, j):
            return x if j < 2 else jnp.concatenate([x[:M], x[8 * j:]], axis=0)

        def spread(y, j):
            filler = jnp.zeros((8, y.shape[1]), F32)
            return y if j < 2 else jnp.concatenate([y[:M]] + [filler] * (j - 1) + [y[M:]], axis=0)

        def group(use, form, half, g):
            p = {q: _dot(use[q], _bf16(form[g, q - 1])) for q in STEP_PRODUCTS[odd]}
            env.setdefault("latest", p[STEP_PRODUCTS[odd][0]])
            m = _memory_out({q: y[:M] for q, y in p.items()}, odd)
            p = {q: p[q][M:] for q in TOKEN_PRODUCTS[odd]}
            if odd:
                return m, _second_half(p, [half[g, k] for k in range(6)])
            for k, z in enumerate(_first_half(p)):
                half[g, k] = z
            return m, ()

        def operands(mark):
            return lhs if mark is None else {p: after(x, env["marks"][mark]) for p, x in lhs.items()}

        def project(side, a0, a1, mark=None):
            form, dst_mem, dst_tok, half = sides[side]
            use = operands(mark)
            for a in range(a0, a1):
                (m0, t0), (m1, t1) = (group(use, form, half, hd) for hd in (2 * a, 2 * a + 1))
                for dt in range(DT):
                    put_rows(lambda j: dst_mem.at[dt], a, m0[dt], m1[dt])
                    for slot, y0, y1 in zip(slots, t0, t1):
                        put_rows(lambda j: dst_tok.at[slot, dt, j], a, y0[dt], y1[dt])

        def project_extras(hf, mark=None):
            def put_memory(column, t):
                kind, a = column[0], 4 * hf + column[1]
                if kind == "q":
                    env["q1", a] = jnp.concatenate([t, q_tok[i, a]], axis=0)
                else:
                    dst = k_mem if kind == "k" else v_mem
                    put_rows(lambda j: dst.at[DT], a, t, pltpu.roll(t, D2, 1))

            use = operands(mark)
            for g, columns in enumerate(EXTRA_GROUPS):
                m, ts = group(use, xform, x_half, len(EXTRA_GROUPS) * hf + g)
                for column, t in zip(columns, m):
                    put_memory(column, t)
                for slot, ys in zip(slots, ts):
                    for column, y in zip(columns, ys):
                        put_extra(slot, hf, column, y)
            plain = jnp.concatenate([h[:M, :D1], ahead[SEG * odd:SEG * odd + SEG, :D1]], axis=0)
            n = len(EXTRA_SINGLES)
            y = _dot(plain, _cat([_bf16(xplain[n * hf + g]) for g in range(n)], 1))
            for g, column in enumerate(EXTRA_SINGLES):
                put_memory(column, _tile(y, g)[:M])
                put_extra(slots[odd], hf, column, _tile(y, g)[M:])

        def query_corner():
            y = _dot(h[:, D1:], _cat([_bf16(wq2[a]) for a in range(HP)], 1))
            for a in range(HP):
                env["q2", a] = _tile(y, a)

        def leftover_scores(a0, a1):
            y = jnp.concatenate(x2g, axis=0)
            for a in range(a0, a1):
                r = _dot(env["q1", a] + env["q2", a], y, NT)
                env["s2", a] = r if a == 0 else pltpu.roll(r, 16 * a, 1)

        def scores(j, wait=0):
            x = live(after(h, env.pop("latest")) if wait else h, j)
            env.pop("latest", None)
            if j == 0:
                kt_mem[...] = _words(k_mem[DT].T[:D2])
                y = _dot(x[:, D1:], _bf16(kt_mem[...]))
                y += _dot(x[:, :D1], _cat([k_mem[dt] for dt in range(DT)], 1), NT)
            else:
                y = _dot(x, _bf16(kt_tok[i, j - 1]))
            env["s", j] = spread(y, j)
            env["marks"].append(env["s", j])

        def turn(k):
            last = [t[min(r + 56, D // 2 - 8):][:8] for t in turn_keys(slots[k]) for r in range(0, D // 2, 64)]
            env["marks"].append(pltpu.bitcast(functools.reduce(jnp.bitwise_or, last) & 0x3FFFFFFF, F32))

        def logits(j):
            w = env["s2", 0]
            for a in range(1, HP):
                w = jnp.where(pair_of_lane == (a + j) % HP, env["s2", a], w)
            w = w if j == 0 else pltpu.roll(w, 128 - 16 * j, 1)
            return jnp.where((row < M) | (row >= 8 * j + (lane & 7)), (env["s", j] + w) * E ** -0.5, NEG)

        def softmax():
            st = [logits(j) for j in range(JB)]
            mx = _reduce_groups(functools.reduce(jnp.maximum, st), jnp.maximum, lane)
            et = [jnp.exp(t - mx) for t in st]
            inv = 1.0 / _reduce_groups(functools.reduce(jnp.add, et), jnp.add, lane)
            env["p"] = [t * inv for t in et]
            env["rolled"] = [t if j == 0 else pltpu.roll(t, 16 * j, 1) for j, t in enumerate(env["p"])]

        def leftover_mix(a0, a1):
            for a in range(a0, a1):
                u = env["rolled"][0]
                for j in range(1, JB):
                    u = jnp.where(pair_of_lane == (a + j) % HP, env["rolled"][j], u)
                env["z", a] = _dot(u, jnp.concatenate([x2g[(q - a) % HP] for q in range(HP)], axis=0))

        def accumulate(y):
            env["o"] = env["o"] + y if "o" in env else y

        def leftover_values(a0, a1):
            w = _cat([_cat([_bf16(wv2[dt, a]) for a in range(a0, a1)], 0) for dt in range(DT + 1)], 1)
            accumulate(_dot(_cat([env["z", a] for a in range(a0, a1)], 1), w[:, :D]))

        def values(j0, j1):
            for j in range(j0, j1):
                v = _cat([v_mem[dt] if j == 0 else v_tok[i, dt, j - 1] for dt in range(DT + 1)], 1)[:, :D]
                accumulate(spread(_dot(live(env["p"][j], j), v), j))

        def mixer(part, mark=None):
            def ordered(g):
                if mark is None:
                    return g
                head = after(g[:16].astype(F32), env["marks"][mark]).astype(BF16)
                return jnp.concatenate([head, g[16:]], axis=0)

            env.setdefault("latest", _tile(mix(part, ordered), 0))

        pieces = {"K": functools.partial(project, "K"), "V": functools.partial(project, "V"), "X": project_extras,
                  "q": query_corner, "t": leftover_scores, "S": scores, "T": turn, "x": softmax,
                  "z": leftover_mix, "b": leftover_values, "P": values, "M": mixer}
        for piece in SCHEDULE[odd].split():
            pieces[piece[0]](*[int(c) for c in piece[1:]])
        return env["o"]

    mix_rows = D // NSEG

    def block(blk, mem):
        @pl.when(blk == 1)
        def _():
            w1_rest.wait()
            w2_all.start()

        always = lax.broadcasted_iota(jnp.int32, (8, 512), 1) > blk - NBLK
        prev = jnp.maximum(blk - 1, 0)
        k0 = pl.multiple_of(prev * BLK, BLK)
        g = mixer_input(prev)
        g_s[...] = jnp.where(blk > 0, g, jnp.zeros_like(g))
        x_next[...] = normalized_tokens(jnp.minimum(blk + 1, NBLK - 1))

        for i in range(NSEG):
            def mix(part, ordered, i=i):
                rows = slice(mix_rows * i, mix_rows * i + mix_rows)
                cols = slice(512 * part, min(512 * part + 512, F))
                y = _dot(ordered(g_s[rows, :]), w1_v[pl.ds(k0, BLK), cols])
                u_s[rows, cols] += y
                return y

            ahead = x_cur[2 * SEG:] if i < 2 else x_next[:2 * SEG]
            o = step(i, jnp.concatenate([mem, x_cur[SEG * i:SEG * i + SEG]], axis=0), ahead, mix, always)
            mem = o[:M]
            o_s[SEG * i:SEG * i + SEG, :] = o[M:]
        x_cur[...] = x_next[...]
        return mem

    lax.fori_loop(0, NBLK, block, mem0_ref[...].astype(F32))

    w2_all.wait()
    hm, hk = D // 2, F // 2
    g = mixer_input(NBLK - 1)
    b1 = b1_ref[...].astype(F32).reshape(1, F)

    def hidden(r, c):
        rows, cols = slice(hm * r, hm * r + hm), slice(hk * c, hk * c + hk)
        u = u_s[rows, cols] + _dot(g[rows], w1_v[S - BLK:, cols]) + b1[:, cols]
        return jax.nn.gelu(u, approximate=True)

    a11 = hidden(0, 0)
    a_s[2] = a11.astype(BF16)
    a12 = hidden(0, 1)
    a_s[4] = (a11 + a12).astype(BF16)
    a21 = hidden(1, 0)
    a_s[5] = (a21 - a11).astype(BF16)
    a22 = hidden(1, 1)
    for k, t in ((3, a22), (1, a21 + a22), (6, a12 - a22), (0, a11 + a22)):
        a_s[k] = t.astype(BF16)

    def emit(y, rows, c0):
        cols = slice(c0, c0 + y.shape[1])
        out_v[rows, cols] = (ht_s[rows, cols] + y + b2_s[0:1, cols]).astype(BF16)

    stores = []
    for c in range(0, S, OUT_COLS):
        w = OUT_COLS // 2
        left, right = slice(c, c + w), slice(c + w, c + OUT_COLS)
        r11, r12, r21, r22 = w2_v[:hk, left], w2_v[:hk, right], w2_v[hk:, left], w2_v[hk:, right]
        b11, b12, b21, b22 = (r.astype(F32) for r in (r11, r12, r21, r22))
        bs = [(b11 + b22).astype(BF16), r11, (b12 - b22).astype(BF16), (b21 - b11).astype(BF16), r22,
              (b11 + b12).astype(BF16), (b21 + b22).astype(BF16)]
        m = {j: _dot(a_s[j], bs[j]) for j in (2, 4, 5, 3, 1, 6, 0)}
        emit(m[2] + m[4], slice(0, hm), c + w)
        emit(m[1] + m[3], slice(hm, D), c)
        emit(m[0] + m[3] - m[4] + m[6], slice(0, hm), c)
        emit(m[0] - m[1] + m[2] + m[5], slice(hm, D), c + w)
        cols = slice(c, c + OUT_COLS)
        stores.append(pltpu.make_async_copy(out_v.at[:, cols], out_hbm.at[:, cols], ysems.at[len(stores)]))
        stores[-1].start()
    for copy in stores:
        copy.wait()


@functools.partial(jax.jit, static_argnames=("A_seg_len",))
def pallas_sequential_preLN__memory_aug_recurrent_mem_tr__mixer_token_mlp__prompt_kernel(
    A_x, A_mem0, A_Wq, A_Wk, A_Wv, A_Wo, A_seg_len, B_x, B_w1, B_b1, B_w2, B_b2
):
    del B_x
    assert A_seg_len == SEG and A_x.shape == (1, S, D) and A_Wq.shape == (D, H, E) and B_w1.shape == (S, F)
    hbm = pl.BlockSpec(memory_space=pl.ANY)
    resident = pl.BlockSpec(memory_space=pltpu.VMEM)
    vmem = pltpu.VMEM
    groups, singles = 2 * len(EXTRA_GROUPS), 2 * len(EXTRA_SINGLES)
    out = pl.pallas_call(
        _kernel,
        out_shape=jax.ShapeDtypeStruct((D, S), BF16),
        in_specs=[hbm, resident, hbm, hbm, hbm, hbm, hbm, resident, hbm, resident],
        out_specs=hbm,
        scratch_shapes=[
            vmem((D, S), BF16),
            vmem((2, D, 8, E), BF16), vmem((2, D, 8, E), BF16), vmem((2, D, 8, E), BF16), vmem((2, 8, D, E), BF16),
            vmem((S, F), BF16), vmem((F, S), BF16),
            vmem((H, NP, 64, 128), U32), vmem((H, NP, 64, 128), U32),
            vmem((groups, NP, 64, 128), U32), vmem((singles, D1 // 2, 128), U32),
            vmem((HP, D2 // 2, 128), U32), vmem((DT + 1, HP, 64, 128), U32),
            vmem((BLK, D), F32), vmem((BLK, D), F32), vmem((BLK, D), F32),
            vmem((D, S), F32), vmem((D, BLK), BF16), vmem((D, F), F32),
            vmem((DT + 1, 128, 128), BF16), vmem((DT + 1, 128, 128), BF16),
            vmem((NSEG, DT + 1, JB - 1, 128, 128), BF16), vmem((NSEG, DT + 1, JB - 1, 128, 128), BF16),
            vmem((NSEG, HP, SEG, 128), F32),
            vmem((H, 6, SEG, 128), F32), vmem((H, 6, SEG, 128), F32), vmem((groups, 6, SEG, 128), F32),
            vmem((D2 // 2, 128), U32), vmem((NSEG, JB - 1, D // 2, 128), U32),
            vmem((7, D // 2, F // 2), BF16), vmem((8, S), F32), vmem((D, S), BF16),
            pltpu.SemaphoreType.DMA((10,)), pltpu.SemaphoreType.DMA((5,)), pltpu.SemaphoreType.DMA((S // OUT_COLS,)),
        ],
        compiler_params=pltpu.CompilerParams(vmem_limit_bytes=110 * 1024 * 1024),
    )(A_x.reshape(S, D).T, A_mem0.reshape(M, D), A_Wq, A_Wk, A_Wv, jnp.transpose(A_Wo, (0, 2, 1)),
      B_w1, B_b1, B_w2, B_b2)
    return out.T.reshape(1, S, D)
```

```python
import functools
import math

import jax
import jax.experimental.pallas as pl
import jax.experimental.pallas.tpu as pltpu
import jax.numpy as jnp
from jax import lax

F32, BF16, U32 = jnp.float32, jnp.bfloat16, jnp.uint32

D = 448
S = 2048
H = 16
E = 256
M = 8
SEG = 32
L = M + SEG
F = 1792
BLK = 128
NSEG = BLK // SEG
NBLK = S // BLK
JB = L // 8
DT = 3
D1 = 128 * DT
D2 = D - D1
HP = H // 2
NP = 15
OUT_COLS = 256
WO_CUTS = (0, 2, 8)
EPS = 1e-5
NEG = -1000000000.0

NT = (((1,), (1,)), ((), ()))
NN = (((1,), (0,)), ((), ()))


def _dot(a, b, dims=NN):
    return lax.dot_general(a, b, dims, preferred_element_type=F32)


def _words(x):
    return pltpu.bitcast(x, U32)


def _bf16(x):
    return pltpu.bitcast(x, BF16)


def _cat(xs, axis):
    return xs[0] if len(xs) == 1 else jnp.concatenate(xs, axis=axis)


def _tile(x, t):
    return x[:, 128 * t:128 * t + 128]


def _tiles(x):
    return [_tile(x, t) for t in range(DT)]


def _layernorm_columns(x):
    m = jnp.sum(x, axis=0, keepdims=True) * (1.0 / D)
    c = x - m
    v = jnp.sum(c * c, axis=0, keepdims=True) * (1.0 / D)
    return c * lax.rsqrt(v + EPS)


def _gelu(u):
    c = (2.0 / math.pi) ** 0.5
    half = 0.5 * u
    return half + half * jnp.tanh(u * (c + (c * 0.044715) * (u * u)))


def _reduce_groups(x, op, lane):
    terms = [x] + [jnp.where(lane % 8 + k < 8, pltpu.roll(x, 128 - k, 1), pltpu.roll(x, 8 - k, 1))
                   for k in range(1, 8)]
    while len(terms) > 1:
        terms = [op(a, b) for a, b in zip(terms[::2], terms[1::2])]
    return terms[0]


def _weight_forms(w):
    (w11, w12, w13), (w21, w22, w23), (w31, w32, w33) = w
    return {1: w11 - w31 - w12, 2: w11 - w21 - w13, 3: w22 - w21 - w32, 4: w22 - w12 - w23, 5: w33 - w31 - w23,
            6: w33 - w32 - w13, 7: w21, 8: w12 - w21, 9: w12, 10: w23, 11: w32 - w23, 12: w32, 13: w13 - w31,
            14: w13, 15: w31}


def _token_forms(a, b):
    (a1, a2, a3), (b1, b2, b3) = a, b
    b12, a23 = b1 + b2, a2 + a3
    return {1: a1, 2: a1 + b1, 3: a2, 4: b2, 5: a3 + b3, 6: b3, 7: a1 + a2 + b12, 8: a1 + b12, 9: b12,
            10: a23 + b2 + b3, 11: a23 + b3, 12: a23, 13: a1 - b3, 14: b1 + b3, 15: a1 + a3}


TOKEN_PRODUCTS = ((1, 3, 5, 7, 9, 10, 12, 15), (2, 4, 6, 8, 11, 13, 14))


def _first_half(p):
    z23 = p[10] - p[12]
    z21 = p[1] - p[9]
    z = [z21 + p[15], p[3] - p[9] + p[12], p[5] + p[12] + p[15], z21, z23 + p[9], z23]
    return [z[0] + p[7], z[1] + p[7]] + z[2:]


def _second_half(p, z):
    t = p[6] + p[11]
    return ([z[0] + p[8], z[1] + p[8], z[2] - t + p[13]],
            [p[2] - p[8] - z[3] + p[13] + p[14], z[4] + p[4] + p[11], z[5] + t + p[14]])


STEP_PRODUCTS = ((1, 3, 5, 10, 9, 7, 12, 13, 15), (2, 7, 6, 8, 4, 11, 13, 10, 14))


def _memory_forms(m, odd):
    m1, m2, m3 = m
    m12, m13, m23 = m1 + m2, m1 + m3, m2 + m3
    if odd:
        return {2: m1, 4: m2, 6: m3, 7: m12, 8: m12, 10: m23, 11: m3, 13: m3, 14: m13}
    return {1: m1, 3: m2, 5: m3, 7: m2, 9: m1, 10: m23, 12: m23, 13: m1, 15: m13}


def _memory_out(p, odd):
    if odd:
        t = p[10] + p[11]
        return [p[2] + p[7] + p[14] - p[13], p[4] + p[7] + p[8] + t, p[6] + p[14] + t]
    t = p[7] + p[9]
    return [p[1] + t + p[15], p[3] + t + p[12], p[5] + p[10] + p[13] + p[15]]


EXTRA_GROUPS = (
    (("k", 0), ("q", 0), ("k", 1)), (("q", 1), ("k", 2), ("q", 2)), (("v", 0), ("v", 1), ("v", 2)),
    (("k", 4), ("q", 4), ("k", 5)), (("q", 5), ("k", 6), ("q", 6)), (("v", 4), ("v", 5), ("v", 6)),
    (("k", 3), ("q", 3), ("k", 7)),
)
EXTRA_SINGLES = (("v", 3), ("v", 7), ("q", 7))
EXTRA_PARTS = (((0, 1, 2), (0,)), ((3, 4, 5, 6), (1, 2)))

SCHEDULE = (
    "q S4 K01 X0 K120 X1 S3 K23 S2 K34 K452 t08 S1 K56 K67 K78 "
    "V013 V12 S01 V24 M0 M2 V45 V56 V68 x M1 z08 P15 P01 b08 M3",
    "K01 X0 K12 K23 S31 q S4 K34 K450 X1 S11 t03 t36 t68 K56 S2 K671 K782 T0 "
    "T1 V013 V12 M0 S0 V23 V346 V454 V56 M16 V675 V78 x M34 z08 P15 P01 b08 M2",
)


def _kernel(xt_hbm, mem0_hbm, wq_hbm, wk_hbm, wv_hbm, wot_hbm, w1_hbm, b1_hbm, w2_hbm, b2_hbm,
            out_hbm,
            xt_v, wq_v, wk_v, wv_v, wot_v, w1_v, w2_v,
            kform, vform, xform, xplain, last_pair, wq2, wv2, x_cur, x_next, o_s, ht_s, g_s, u_s,
            k_mem, v_mem, k_tok, v_tok, q_tok, k_half, v_half, x_half, kt_mem, kt_tok, a_s, b2_s, out_v,
            mem0_v, b1_v, b2_v, wsems, lsems, ysems):
    def heads(hf):
        return pl.ds(pl.multiple_of(8 * hf, 8), 8)

    def value_copies(hf):
        return [pltpu.make_async_copy(wv_hbm.at[:, heads(hf), :], wv_v.at[hf], wsems.at[5 * hf])] + [
            pltpu.make_async_copy(wot_hbm.at[pl.ds(8 * hf + h0, h1 - h0)], wot_v.at[hf, pl.ds(h0, h1 - h0)],
                                  wsems.at[5 * hf + 3 + c]) for c, (h0, h1) in enumerate(zip(WO_CUTS, WO_CUTS[1:]))]

    def key_copies(hf):
        return [pltpu.make_async_copy(wq_hbm.at[:, heads(hf), :], wq_v.at[hf], wsems.at[5 * hf + 1]),
                pltpu.make_async_copy(wk_hbm.at[:, heads(hf), :], wk_v.at[hf], wsems.at[5 * hf + 2])]

    x_head = pltpu.make_async_copy(xt_hbm.at[:, pl.ds(0, BLK)], xt_v.at[:, pl.ds(0, BLK)], lsems.at[0])
    x_rest = pltpu.make_async_copy(xt_hbm.at[:, pl.ds(BLK, S - BLK)], xt_v.at[:, pl.ds(BLK, S - BLK)], lsems.at[1])
    w1_head = pltpu.make_async_copy(w1_hbm.at[pl.ds(0, BLK)], w1_v.at[pl.ds(0, BLK)], lsems.at[2])
    w1_rest = pltpu.make_async_copy(w1_hbm.at[pl.ds(BLK, S - BLK)], w1_v.at[pl.ds(BLK, S - BLK)], lsems.at[3])
    w2_all = pltpu.make_async_copy(w2_hbm, w2_v, lsems.at[4])
    small = [pltpu.make_async_copy(src, dst, lsems.at[5 + k])
             for k, (src, dst) in enumerate(((b1_hbm, b1_v), (b2_hbm, b2_v), (mem0_hbm, mem0_v)))]
    queue = [x_head] + small + value_copies(0) + value_copies(1) + key_copies(0) + key_copies(1) + [x_rest, w1_head]

    def request(i, carry):
        for k, copy in enumerate(queue):
            pl.when(i == k)(copy.start)
        return carry

    lax.fori_loop(0, len(queue), request, 0)
    x_head.wait()
    for copy in small:
        copy.wait()

    def start_from_bias(i, carry):
        u_s[pl.ds(pl.multiple_of(i * 32, 32), 32), :] = jnp.broadcast_to(b1_v[...].astype(F32).reshape(1, F), (32, F))
        return carry

    lax.fori_loop(0, D // 32, start_from_bias, 0)
    o_s[...] = jnp.zeros(o_s.shape, F32)
    b2_s[...] = jnp.broadcast_to(b2_v[...].astype(F32).reshape(1, S), b2_s.shape)

    def by_head(w):
        w = jnp.swapaxes(w, 0, 1)
        return [w[hd] for hd in range(8)]

    def put_forms(form, i, columns):
        blocks = [[c[128 * k:128 * k + 128] for c in columns] for k in range(DT)]
        for p, t in _weight_forms(blocks).items():
            form[i, p - 1] = _words(t.astype(BF16))

    def fold_pair(ls, rs, a, form):
        rp = jnp.concatenate([r[D1:] for r in rs], axis=0)
        lane = lax.broadcasted_iota(jnp.int32, (D, 128), 1)
        shared = jnp.where(lane < D2, *[_dot(l, rp, NT) for l in ls])
        full = [_dot(l, r[:D1], NT) for l, r in zip(ls, rs)]
        for b, y in enumerate(full):
            put_forms(form, 2 * a + b, _tiles(y))
        tails = [jnp.concatenate([_tile(y[D1:], dt) for y in full], axis=0) for dt in range(DT)]
        tails.append(jnp.concatenate([shared[D1:], pltpu.roll(shared[D1:], D2, 1)], axis=0))
        return shared[:D1], [t.astype(BF16) for t in tails]

    def fold_values(hf, carry):
        arrivals = value_copies(hf)
        arrivals[0].wait()
        wv = by_head(wv_v[hf])
        extras = {}
        for k in range(HP // 2):
            a = 4 * hf + k
            if 2 * k in WO_CUTS:
                arrivals[1 + WO_CUTS.index(2 * k)].wait()
            extras["v", k], tails = fold_pair(wv[2 * k:2 * k + 2], [wot_v[hf, 2 * k + b] for b in range(2)], a, vform)
            for dt, t in enumerate(tails):
                wv2[dt, a] = _words(t)
        put_forms(xform, 3 * hf + 2, [extras[c] for c in EXTRA_GROUPS[2]])
        xplain[hf] = _words(extras["v", 3].astype(BF16))
        return carry

    def fold_keys(hf, carry):
        for copy in key_copies(hf):
            copy.wait()
        wq, wk = by_head(wq_v[hf]), by_head(wk_v[hf])
        extras = {}
        for k in (3, 0, 1, 2):
            a = 4 * hf + k
            extras["k", k], tails = fold_pair(wk[2 * k:2 * k + 2], wq[2 * k:2 * k + 2], a, kform)
            extras["q", k] = jnp.concatenate([t.T.astype(F32) for t in tails[:DT]], axis=0)
            wq2[a] = _words(tails[DT].T[:D2])
        for g in range(2):
            put_forms(xform, 3 * hf + g, [extras[c] for c in EXTRA_GROUPS[g]])
        last_pair[hf, 0] = extras["k", 3]
        last_pair[hf, 1] = extras["q", 3]
        first_tokens("K", hf)
        return carry

    def normalized_tokens(blk):
        c0 = pl.multiple_of(blk * BLK, BLK)
        return _layernorm_columns(xt_v[:, pl.ds(c0, BLK)].astype(F32)).astype(BF16).T.astype(F32)

    def mixer_input(blk):
        c0 = pl.multiple_of(blk * BLK, BLK)
        h = xt_v[:, pl.ds(c0, BLK)].astype(F32) + o_s[...].T
        ht_s[:, pl.ds(c0, BLK)] = h + b2_s[0:1, pl.ds(c0, BLK)]
        return _layernorm_columns(_layernorm_columns(h)).astype(BF16)

    def put_rows(dst, a, y0, y1):
        for j in range(y0.shape[0] // 8):
            t = jnp.concatenate([y0[8 * j:8 * j + 8], y1[8 * j:8 * j + 8]], axis=0).astype(BF16)
            dst(j)[pl.ds(pl.multiple_of(16 * a, 16), 16), :] = t

    def put_extra(slot, column, y):
        kind, a = column
        if kind == "q":
            q_tok[slot, a] = y
        else:
            dst = k_tok if kind == "k" else v_tok
            put_rows(lambda j: dst.at[slot, DT, j], a, y, pltpu.roll(y, D2, 1))

    def turn_keys(slot):
        ts = [_words(_cat([k_tok[slot, dt, j].T for dt in range(DT + 1)], 0)[:D]) for j in range(JB - 1)]
        for j, t in enumerate(ts):
            kt_tok[slot, j] = t
        return ts

    sides = {"K": (kform, k_mem, k_tok, k_half), "V": (vform, v_mem, v_tok, v_half)}

    def first_tokens(side, hf):
        tok = _token_forms(_tiles(x_cur[:SEG]), _tiles(x_cur[SEG:2 * SEG]))

        def project(form, blocks):
            ys = {q: _dot(tok[q], _cat([_bf16(form[i, q - 1]) for i in blocks], 1)) for q in tok}
            ps = [{q: _tile(y, k) for q, y in ys.items()} for k in range(len(blocks))]
            return [_second_half(p, _first_half(p)) for p in ps]

        if side == "X":
            groups, singles = EXTRA_PARTS[hf]
            for g in groups:
                for slot, ys in enumerate(project(xform, [g])[0]):
                    for column, y in zip(EXTRA_GROUPS[g], ys):
                        put_extra(slot, column, y)
            for g in singles:
                y = _dot(x_cur[:2 * SEG, :D1], _bf16(xplain[g]))
                for slot in range(2):
                    put_extra(slot, EXTRA_SINGLES[g], y[SEG * slot:SEG * slot + SEG])
            return
        form, _, dst, _ = sides[side]
        for k in range(HP // 2):
            a = 4 * hf + k
            ys = project(form, [2 * a, 2 * a + 1])
            for slot in range(2):
                for dt in range(DT):
                    put_rows(lambda j: dst.at[slot, dt, j], a, ys[0][slot][dt], ys[1][slot][dt])

    x_cur[...] = normalized_tokens(0)
    lax.fori_loop(0, 2, fold_values, 0)
    lax.fori_loop(0, 2, fold_keys, 0)
    put_forms(xform, 6, [last_pair[0, 0], last_pair[0, 1], last_pair[1, 0]])
    xplain[2] = _words(last_pair[1, 1].astype(BF16))
    for hf in range(2):
        first_tokens("X", hf)
    for hf in range(2):
        first_tokens("V", hf)
    for slot in range(2):
        turn_keys(slot)
    x_rest.wait()
    w1_head.wait()
    w1_rest.start()

    lane = lax.broadcasted_iota(jnp.int32, (L, 128), 1)
    row = lax.broadcasted_iota(jnp.int32, (L, 128), 0)
    pair_of_lane = lane >> 4

    def step(i, h, ahead, mix, always):
        odd = i % 2
        slots = [(i - odd + 2) % NSEG, (i - odd + 3) % NSEG]
        tok = _token_forms(_tiles(ahead[:SEG]), _tiles(ahead[SEG:]))
        mem = _memory_forms(_tiles(h[:M]), odd)
        lhs = {p: jnp.concatenate([mem[p], tok[p]], axis=0) if p in TOKEN_PRODUCTS[odd] else mem[p] for p in mem}
        x2 = jnp.concatenate([h[:, D1:], jnp.zeros((L, 128 - D2), F32)], axis=1)
        x2r = pltpu.roll(x2, D2, 1)
        x2g = [jnp.concatenate([x2[8 * j:8 * j + 8], x2r[8 * j:8 * j + 8]], axis=0).astype(BF16)
               for j in range(JB)] + [jnp.zeros((16, 128), BF16)] * (HP - JB)
        env = {"marks": []}

        def after(x, dep):
            n = -(-x.shape[1] // 128)
            head = jnp.where(always[:, :x.shape[1]], x[:8], _cat([dep[:8]] * n, 1)[:, :x.shape[1]])
            return jnp.concatenate([head, x[8:]], axis=0) if x.shape[0] > 8 else head

        def live(x, j):
            return x if j < 2 else jnp.concatenate([x[:M], x[8 * j:]], axis=0)

        def spread(y, j):
            filler = jnp.zeros((8, y.shape[1]), F32)
            return y if j < 2 else jnp.concatenate([y[:M]] + [filler] * (j - 1) + [y[M:]], axis=0)

        def products(use, form, blocks):
            ys = {q: _dot(use[q], _cat([_bf16(form[g, q - 1]) for g in blocks], 1)) for q in STEP_PRODUCTS[odd]}
            return [{q: _tile(y, k) for q, y in ys.items()} for k in range(len(blocks))]

        def group(p, half, g):
            env.setdefault("latest", p[STEP_PRODUCTS[odd][0]])
            m = _memory_out({q: y[:M] for q, y in p.items()}, odd)
            p = {q: p[q][M:] for q in TOKEN_PRODUCTS[odd]}
            if odd:
                return m, _second_half(p, [half[g, k] for k in range(6)])
            for k, z in enumerate(_first_half(p)):
                half[g, k] = z
            return m, ()

        def operands(mark):
            return lhs if mark is None else {p: after(x, env["marks"][mark]) for p, x in lhs.items()}

        def project(side, a0, a1, mark=None):
            form, dst_mem, dst_tok, half = sides[side]
            use = operands(mark)
            for a in range(a0, a1):
                if odd:
                    both = (group(*products(use, form, [hd]), half, hd) for hd in (2 * a, 2 * a + 1))
                else:
                    both = (group(p, half, 2 * a + b) for b, p in enumerate(products(use, form, [2 * a, 2 * a + 1])))
                (m0, t0), (m1, t1) = both
                for dt in range(DT):
                    put_rows(lambda j: dst_mem.at[dt], a, m0[dt], m1[dt])
                    for slot, y0, y1 in zip(slots, t0, t1):
                        put_rows(lambda j: dst_tok.at[slot, dt, j], a, y0[dt], y1[dt])

        def project_extras(part, mark=None):
            def put_memory(column, t):
                kind, a = column
                if kind == "q":
                    env["q1", a] = jnp.concatenate([t, q_tok[i, a]], axis=0)
                else:
                    dst = k_mem if kind == "k" else v_mem
                    put_rows(lambda j: dst.at[DT], a, t, pltpu.roll(t, D2, 1))

            use = operands(mark)
            groups, singles = EXTRA_PARTS[part]
            for g in groups:
                m, ts = group(*products(use, xform, [g]), x_half, g)
                for column, t in zip(EXTRA_GROUPS[g], m):
                    put_memory(column, t)
                for slot, ys in zip(slots, ts):
                    for column, y in zip(EXTRA_GROUPS[g], ys):
                        put_extra(slot, column, y)
            plain = jnp.concatenate([h[:M, :D1], ahead[SEG * odd:SEG * odd + SEG, :D1]], axis=0)
            y = _dot(plain, _cat([_bf16(xplain[g]) for g in singles], 1))
            for k, g in enumerate(singles):
                put_memory(EXTRA_SINGLES[g], _tile(y, k)[:M])
                put_extra(slots[odd], EXTRA_SINGLES[g], _tile(y, k)[M:])

        def query_corner():
            y = _dot(h[:, D1:], _cat([_bf16(wq2[a]) for a in range(HP)], 1))
            for a in range(HP):
                env["q2", a] = _tile(y, a)

        def leftover_scores(a0, a1):
            y = jnp.concatenate(x2g, axis=0)
            for a in range(a0, a1):
                r = _dot(env["q1", a] + env["q2", a], y, NT)
                env["s2", a] = r if a == 0 else pltpu.roll(r, 16 * a, 1)

        def scores(j, wait=0):
            x = live(after(h, env.pop("latest")) if wait else h, j)
            env.pop("latest", None)
            if j == 0:
                kt_mem[...] = _words(k_mem[DT].T[:D2])
                y = _dot(x[:, D1:], _bf16(kt_mem[...]))
                y += _dot(x[:, :D1], _cat([k_mem[dt] for dt in range(DT)], 1), NT)
            else:
                y = _dot(x, _bf16(kt_tok[i, j - 1]))
            env["s", j] = spread(y, j)
            env["marks"].append(env["s", j])

        def turn(k):
            last = [t[min(r + 56, D // 2 - 8):][:8] for t in turn_keys(slots[k]) for r in range(0, D // 2, 64)]
            env["marks"].append(pltpu.bitcast(functools.reduce(jnp.bitwise_or, last) & 0x3FFFFFFF, F32))

        def logits(j):
            w = env["s2", 0]
            for a in range(1, HP):
                w = jnp.where(pair_of_lane == (a + j) % HP, env["s2", a], w)
            w = w if j == 0 else pltpu.roll(w, 128 - 16 * j, 1)
            return jnp.where((row < M) | (row >= 8 * j + (lane & 7)), (env["s", j] + w) * E ** -0.5, NEG)

        def softmax():
            st = [logits(j) for j in range(JB)]
            mx = _reduce_groups(functools.reduce(jnp.maximum, st), jnp.maximum, lane)
            et = [jnp.exp(t - mx) for t in st]
            inv = 1.0 / _reduce_groups(functools.reduce(jnp.add, et), jnp.add, lane)
            env["p"] = [t * inv for t in et]
            env["rolled"] = [t if j == 0 else pltpu.roll(t, 16 * j, 1) for j, t in enumerate(env["p"])]

        def leftover_mix(a0, a1):
            for a in range(a0, a1):
                u = env["rolled"][0]
                for j in range(1, JB):
                    u = jnp.where(pair_of_lane == (a + j) % HP, env["rolled"][j], u)
                env["z", a] = _dot(u, jnp.concatenate([x2g[(q - a) % HP] for q in range(HP)], axis=0))

        def accumulate(y):
            env["o"] = env["o"] + y if "o" in env else y

        def leftover_values(a0, a1):
            w = _cat([_cat([_bf16(wv2[dt, a]) for a in range(a0, a1)], 0) for dt in range(DT + 1)], 1)
            accumulate(_dot(_cat([env["z", a] for a in range(a0, a1)], 1), w[:, :D]))

        def values(j0, j1):
            for j in range(j0, j1):
                v = _cat([v_mem[dt] if j == 0 else v_tok[i, dt, j - 1] for dt in range(DT + 1)], 1)[:, :D]
                accumulate(spread(_dot(live(env["p"][j], j), v), j))

        def mixer(part, mark=None):
            def ordered(g):
                if mark is None:
                    return g
                head = after(g[:16].astype(F32), env["marks"][mark]).astype(BF16)
                return jnp.concatenate([head, g[16:]], axis=0)

            env.setdefault("latest", _tile(mix(part, ordered), 0))

        pieces = {"K": functools.partial(project, "K"), "V": functools.partial(project, "V"), "X": project_extras,
                  "q": query_corner, "t": leftover_scores, "S": scores, "T": turn, "x": softmax,
                  "z": leftover_mix, "b": leftover_values, "P": values, "M": mixer}
        for piece in SCHEDULE[odd].split():
            pieces[piece[0]](*[int(c) for c in piece[1:]])
        return env["o"]

    mix_rows = D // NSEG

    def block(blk, mem):
        @pl.when(blk == 1)
        def _():
            w1_rest.wait()
            w2_all.start()

        always = lax.broadcasted_iota(jnp.int32, (8, 512), 1) > blk - NBLK
        prev = jnp.maximum(blk - 1, 0)
        k0 = pl.multiple_of(prev * BLK, BLK)
        g = mixer_input(prev)
        g_s[...] = jnp.where(blk > 0, g, jnp.zeros_like(g))
        x_next[...] = normalized_tokens(jnp.minimum(blk + 1, NBLK - 1))

        for i in range(NSEG):
            def mix(part, ordered, i=i):
                rows = slice(mix_rows * i, mix_rows * i + mix_rows)
                cols = slice(512 * part, min(512 * part + 512, F))
                y = _dot(ordered(g_s[rows, :]), w1_v[pl.ds(k0, BLK), cols])
                u_s[rows, cols] += y
                return y

            ahead = x_cur[2 * SEG:] if i < 2 else x_next[:2 * SEG]
            o = step(i, jnp.concatenate([mem, x_cur[SEG * i:SEG * i + SEG]], axis=0), ahead, mix, always)
            mem = o[:M]
            o_s[SEG * i:SEG * i + SEG, :] = o[M:]
            if i:
                done = slice(0 if i == 1 else SEG * i, SEG * i + SEG)
                x_cur[done] = x_next[done]
        return mem

    lax.fori_loop(0, NBLK, block, mem0_v[...].astype(F32))

    w2_all.wait()
    hm, hk = D // 2, F // 2
    g = mixer_input(NBLK - 1)

    def hidden(c):
        cols = slice(hk * c, hk * c + hk)
        y = _dot(g, w1_v[S - BLK:, cols])
        return [_gelu(u_s[rows, cols] + y[rows]) for rows in (slice(0, hm), slice(hm, D))]

    a11, a21 = hidden(0)
    a_s[2] = a11.astype(BF16)
    a_s[5] = (a21 - a11).astype(BF16)
    a12, a22 = hidden(1)
    a_s[4] = (a11 + a12).astype(BF16)
    for k, t in ((3, a22), (1, a21 + a22), (6, a12 - a22), (0, a11 + a22)):
        a_s[k] = t.astype(BF16)

    def emit(y, rows, c0):
        cols = slice(c0, c0 + y.shape[1])
        out_v[rows, cols] = (ht_s[rows, cols] + y).astype(BF16)

    stores = []

    def send(cols):
        stores.append(pltpu.make_async_copy(out_v.at[:, cols], out_hbm.at[:, cols], ysems.at[len(stores)]))
        stores[-1].start()

    for c in range(0, S, OUT_COLS):
        w = OUT_COLS // 2
        left, right = slice(c, c + w), slice(c + w, c + OUT_COLS)
        r11, r12, r21, r22 = w2_v[:hk, left], w2_v[:hk, right], w2_v[hk:, left], w2_v[hk:, right]
        b11, b12, b21, b22 = (r.astype(F32) for r in (r11, r12, r21, r22))
        bs = [(b11 + b22).astype(BF16), r11, (b12 - b22).astype(BF16), (b21 - b11).astype(BF16), r22,
              (b11 + b12).astype(BF16), (b21 + b22).astype(BF16)]
        last = c + OUT_COLS == S
        m = {j: _dot(a_s[j], bs[j]) for j in ((3, 6, 1, 4, 0, 2, 5) if last else (2, 4, 1, 3, 0, 6, 5))}
        emit(m[1] + m[3], slice(hm, D), c)
        emit(m[0] + m[3] - m[4] + m[6], slice(0, hm), c)
        if last:
            send(left)
        emit(m[2] + m[4], slice(0, hm), c + w)
        emit(m[0] - m[1] + m[2] + m[5], slice(hm, D), c + w)
        send(right if last else slice(c, c + OUT_COLS))
    for copy in stores:
        copy.wait()


@functools.partial(jax.jit, static_argnames=("A_seg_len",))
def pallas_sequential_preLN__memory_aug_recurrent_mem_tr__mixer_token_mlp__prompt_kernel(
    A_x, A_mem0, A_Wq, A_Wk, A_Wv, A_Wo, A_seg_len, B_x, B_w1, B_b1, B_w2, B_b2
):
    del B_x
    assert A_seg_len == SEG and A_x.shape == (1, S, D) and A_Wq.shape == (D, H, E) and B_w1.shape == (S, F)
    hbm = pl.BlockSpec(memory_space=pl.ANY)
    vmem = pltpu.VMEM
    groups, singles = len(EXTRA_GROUPS), len(EXTRA_SINGLES)
    out = pl.pallas_call(
        _kernel,
        out_shape=jax.ShapeDtypeStruct((D, S), BF16),
        in_specs=[hbm] * 10,
        out_specs=hbm,
        scratch_shapes=[
            vmem((D, S), BF16),
            vmem((2, D, 8, E), BF16), vmem((2, D, 8, E), BF16), vmem((2, D, 8, E), BF16), vmem((2, 8, D, E), BF16),
            vmem((S, F), BF16), vmem((F, S), BF16),
            vmem((H, NP, 64, 128), U32), vmem((H, NP, 64, 128), U32),
            vmem((groups, NP, 64, 128), U32), vmem((singles, D1 // 2, 128), U32), vmem((2, 2, D1, 128), F32),
            vmem((HP, D2 // 2, 128), U32), vmem((DT + 1, HP, 64, 128), U32),
            vmem((BLK, D), F32), vmem((BLK, D), F32), vmem((BLK, D), F32),
            vmem((D, S), F32), vmem((D, BLK), BF16), vmem((D, F), F32),
            vmem((DT + 1, 128, 128), BF16), vmem((DT + 1, 128, 128), BF16),
            vmem((NSEG, DT + 1, JB - 1, 128, 128), BF16), vmem((NSEG, DT + 1, JB - 1, 128, 128), BF16),
            vmem((NSEG, HP, SEG, 128), F32),
            vmem((H, 6, SEG, 128), F32), vmem((H, 6, SEG, 128), F32), vmem((groups, 6, SEG, 128), F32),
            vmem((D2 // 2, 128), U32), vmem((NSEG, JB - 1, D // 2, 128), U32),
            vmem((7, D // 2, F // 2), BF16), vmem((8, S), F32), vmem((D, S), BF16),
            vmem((M, D), BF16), vmem((F,), BF16), vmem((S,), BF16),
            pltpu.SemaphoreType.DMA((10,)), pltpu.SemaphoreType.DMA((8,)), pltpu.SemaphoreType.DMA((S // OUT_COLS + 1,)),
        ],
        compiler_params=pltpu.CompilerParams(vmem_limit_bytes=110 * 1024 * 1024),
    )(A_x.reshape(S, D).T, A_mem0.reshape(M, D), A_Wq, A_Wk, A_Wv, jnp.transpose(A_Wo, (0, 2, 1)),
      B_w1, B_b1, B_w2, B_b2)
    return out.T.reshape(1, S, D)
```
